```python
import os as _os
_os.environ.setdefault("JAX_PLATFORMS", "cpu")
import jax
import jax.numpy as jnp

def _softmax(x, axis=-1):
    return jax.nn.softmax(x, axis=axis)
def _gelu(x):
    return jax.nn.gelu(x, approximate=True)
def _silu(x):
    return jax.nn.silu(x)
def _sigmoid(x):
    return jax.nn.sigmoid(x)
def _layernorm(x, axis=-1, eps=1e-5):
    m = jnp.mean(x, axis=axis, keepdims=True)
    v = jnp.var(x, axis=axis, keepdims=True)
    return (x - m) / jnp.sqrt(v + eps)
def _scatter_add(tgt, idx, src, axis=0):
    return tgt.at[idx].add(src)
def _segment_sum(src, seg, n):
    return jax.ops.segment_sum(src, seg, n)
class _Rng:
    def __init__(self, key):
        self._k = key
    def _next(self):
        self._k, sub = jax.random.split(self._k)
        return sub
    def normal(self, shape):
        return jax.random.normal(self._next(), shape, dtype=jnp.bfloat16)
    def randint(self, lo, hi, shape):
        return jax.random.randint(self._next(), shape, lo, hi, dtype=jnp.int32)
    def uniform(self, shape, lo=0.0, hi=1.0):
        return jax.random.uniform(self._next(), shape, jnp.bfloat16, lo, hi)
    def permutation(self, n):
        return jax.random.permutation(self._next(), n)


kernel_name = 'concat_heads__gqa_block_cached__gqa_block_cached__near_ridge'

def setup_inputs():
    _rng = _Rng(jax.random.key(int.from_bytes(__import__("os").urandom(4), "little")))
    _w = (lambda a: (lambda t: t.astype(jnp.bfloat16) if jnp.issubdtype(t.dtype, jnp.floating) else t)(jnp.asarray(a)))
    def _A_setup():
        B, Sq, D = 8, 128, 576
        Hq, Hkv, Sk, Dh = 32, 16, 512, 128
        assert Hq % Hkv == 0, (Hq, Hkv)
        return {
            "x": _w((lambda *s: _rng.normal(s) * 0.8)(B, Sq, D)),
            "k_cache": _w((lambda *s: _rng.normal(s) * 0.8)(B, Hkv, Sk, Dh)),
            "v_cache": _w((lambda *s: _rng.normal(s) * 0.05)(B, Hkv, Sk, Dh)),
            "wq": _w((lambda *s: _rng.normal(s) * 0.8)(D, Hq * Dh) * (D ** -0.5)),
            "wo": _w((lambda *s: _rng.normal(s) * 0.05)(Hq * Dh, D) * ((Hq * Dh) ** -0.5)),
        }
    _A_in = _A_setup()

    def _B_setup():
        B, Sq, D = 8, 128, 576
        Hq, Hkv, Sk, Dh = 32, 16, 512, 128
        assert Hq % Hkv == 0, (Hq, Hkv)
        return {
            "x": _w((lambda *s: _rng.normal(s) * 0.8)(B, Sq, D)),
            "k_cache": _w((lambda *s: _rng.normal(s) * 0.8)(B, Hkv, Sk, Dh)),
            "v_cache": _w((lambda *s: _rng.normal(s) * 0.05)(B, Hkv, Sk, Dh)),
            "wq": _w((lambda *s: _rng.normal(s) * 0.8)(D, Hq * Dh) * (D ** -0.5)),
            "wo": _w((lambda *s: _rng.normal(s) * 0.05)(Hq * Dh, D) * ((Hq * Dh) ** -0.5)),
        }
    _B_in = _B_setup()

    return {
        "A_x": _A_in["x"],
        "A_k_cache": _A_in["k_cache"],
        "A_v_cache": _A_in["v_cache"],
        "A_wq": _A_in["wq"],
        "A_wo": _A_in["wo"],
        "B_x": _B_in["x"],
        "B_k_cache": _B_in["k_cache"],
        "B_v_cache": _B_in["v_cache"],
        "B_wq": _B_in["wq"],
        "B_wo": _B_in["wo"],
    }

def reference(A_x, A_k_cache, A_v_cache, A_wq, A_wo, B_x, B_k_cache, B_v_cache, B_wq, B_wo):
    def _A_ref(x, k_cache, v_cache, wq, wo):
        B, Sq, D = x.shape
        Hq, Dh = 32, 128
        Hkv = k_cache.shape[1]
        rep = Hq // Hkv
        q = (lambda x, *d: x.transpose(*d))((x @ wq).reshape(B, Sq, Hq, Dh), 0, 2, 1, 3)
        k = jnp.repeat(k_cache, rep, axis=1)
        v = jnp.repeat(v_cache, rep, axis=1)
        scores = jnp.einsum("bhqd,bhkd->bhqk", q, k) * (Dh ** -0.5)
        p = _softmax(scores, axis=-1)
        o = jnp.einsum("bhqk,bhkd->bhqd", p, v)
        return (lambda x, *d: x.transpose(*d))(o, 0, 2, 1, 3).reshape(B, Sq, Hq * Dh) @ wo

    def _B_ref(x, k_cache, v_cache, wq, wo):
        B, Sq, D = x.shape
        Hq, Dh = 32, 128
        Hkv = k_cache.shape[1]
        rep = Hq // Hkv
        q = (lambda x, *d: x.transpose(*d))((x @ wq).reshape(B, Sq, Hq, Dh), 0, 2, 1, 3)
        k = jnp.repeat(k_cache, rep, axis=1)
        v = jnp.repeat(v_cache, rep, axis=1)
        scores = jnp.einsum("bhqd,bhkd->bhqk", q, k) * (Dh ** -0.5)
        p = _softmax(scores, axis=-1)
        o = jnp.einsum("bhqk,bhkd->bhqd", p, v)
        return (lambda x, *d: x.transpose(*d))(o, 0, 2, 1, 3).reshape(B, Sq, Hq * Dh) @ wo

    a = _A_ref(A_x, A_k_cache, A_v_cache, A_wq, A_wo)
    b = _B_ref(B_x, B_k_cache, B_v_cache, B_wq, B_wo)
    return jnp.concatenate([a, b], axis=-1)
```

```python
import numpy as np
import jax
import jax.numpy as jnp
from jax import lax
import jax.experimental.pallas as pl
import jax.experimental.pallas.tpu as pltpu
import contextlib

B, SQ, D = 8, 128, 576
HQ, HKV, SK, DH = 32, 16, 512, 128
M = B * SQ
GW = 2 * DH
NSTEP = 2 * HKV
AHEAD = int('2')
NQ = 8
U = int("2")
OD = int(str(U))
NS = max(2 * U, 2)
NW = 8
NP = max(U, OD)
HCH = int("1")
LO = 512
HI = 2 * D - LO
LOG2E = 1.4426950408889634
QSCALE = float((DH ** -0.5) * LOG2E)
NT = (((1,), (1,)), ((), ()))
FLAGS = ""
FLOAT = "RESCHEDULE" in FLAGS
SC = "0"
ATT = "W Q0 Q1 P0 Q2 P1 Q3 P2 Q4 P3 Q5 P4 Q6 P5 Q7 P6 P7"
ATT0 = "W0 Q0 Q1 P0 Q2 P1 Q3 P2 W1 Q4 P3 Q5 P4 Q6 P5 Q7 P6 P7"
ORDER = "O0 D B O1 O2 O3 " + ATT + " X0 X1"
ORDER1 = ORDER
ORDER_0 = "D " + ATT0 + " X0 X1"
ORDER_P = "D " + ATT + " X0 X1"
ORDER_T = "O0 D O1 A O2 O3 " + ATT


def scope(n):
    return jax.named_scope(n) if (SC == "1" or (SC == "2" and n != "wait")) else contextlib.nullcontext()


def _kernel(xa, ka, va, wqa, woa, xb, kb, vb, wqb, wob, out,
            xt_buf, x_buf, wq_buf, k_buf, v_buf, wo_buf, q_buf, o_a, o_b, acc, ob_lo, ob_hi,
            sems):
    srcs = ((xa, ka, va, wqa, woa), (xb, kb, vb, wqb, wob))
    o_bufs = (o_a, o_b)
    S_X, S_LO, S_H, S_HI = 0, 3, 4, 8
    S_WQ = S_HI + B
    S_K = S_WQ + NW
    S_V = S_K + NS
    S_WO = S_V + NS

    def xa_copy(h):
        return pltpu.make_async_copy(xa.at[pl.ds(4 * h, 4)], xt_buf.at[0, pl.ds(4 * h, 4)], sems.at[S_X + h])

    def xb_copy():
        return pltpu.make_async_copy(xb, xt_buf.at[1], sems.at[S_X + 2])

    def cols(g):
        return pl.ds(pl.multiple_of(g * GW, GW), GW) if not isinstance(g, int) else pl.ds(g * GW, GW)

    def wq_copy(r, g, slot):
        return pltpu.make_async_copy(srcs[r][3].at[:, cols(g)], wq_buf.at[slot], sems.at[S_WQ + slot])

    def k_copy(r, g, slot):
        return pltpu.make_async_copy(srcs[r][1].at[:, g], k_buf.at[slot], sems.at[S_K + slot])

    def v_copy(r, g, slot):
        return pltpu.make_async_copy(srcs[r][2].at[:, g], v_buf.at[slot], sems.at[S_V + slot])

    def kv0_copy(which, h):
        src, dst = ((ka, k_buf), (va, v_buf))[which]
        return pltpu.make_async_copy(src.at[pl.ds(4 * h, 4), 0], dst.at[0, pl.ds(4 * h, 4)], sems.at[S_H + 2 * h + which])

    def wo_copy(r, g, slot):
        return pltpu.make_async_copy(srcs[r][4].at[:, cols(g)], wo_buf.at[slot], sems.at[S_WO + slot])

    def lo_copy():
        return pltpu.make_async_copy(ob_lo, out.at[:, pl.ds(0, LO)], sems.at[S_LO])

    def hi_copy(b):
        rows = pl.ds(b * SQ * HCH, SQ * HCH)
        return pltpu.make_async_copy(ob_hi.at[rows], out.at[rows, pl.ds(LO, HI)], sems.at[S_HI + b])

    def start(copy, t, slot):
        if isinstance(t, int):
            if 0 <= t < NSTEP:
                copy(t >> 4, t & (HKV - 1), slot).start()
            return
        r = lax.shift_right_logical(t, 4)
        g = t & (HKV - 1)
        for rr in range(2):
            @pl.when(r == rr)
            def _():
                copy(rr, g, slot).start()

    def prefetch(s):
        start(k_copy, s + U, (s + U) & (NS - 1))
        start(v_copy, s + U, (s + U) & (NS - 1))
        start(wq_copy, s + U + AHEAD, (s + U + AHEAD) & (NW - 1))
        start(wo_copy, s + U - OD, (s + U - OD) & (NS - 1))

    def xpose(src_r, dst_r, b):
        rows = pl.ds(b * SQ, SQ) if isinstance(b, int) else pl.ds(pl.multiple_of(b * SQ, SQ), SQ)
        x_buf[dst_r, rows, :] = xt_buf[src_r, b].T

    def qproj(r, wslot, qslot, r0, n):
        q = jnp.dot(x_buf[r, pl.ds(r0, n), :], wq_buf[wslot], preferred_element_type=jnp.float32)
        q_buf[qslot, pl.ds(r0, n), :] = (q * QSCALE).astype(jnp.bfloat16)

    def has(order, c):
        return any(t[0] == c for t in order.split())

    def waits(s, order):
        if has(order, "Q") and "W0" not in order.split():
            k_copy(0, 0, s & (NS - 1)).wait()
            v_copy(0, 0, s & (NS - 1)).wait()
        if has(order, "O"):
            wo_copy(0, 0, (s - OD) & (NS - 1)).wait()
        if has(order, "X"):
            wq_copy(0, 0, (s + AHEAD) & (NW - 1)).wait()

    def events(s0):
        @pl.when(s0 == 2)
        def _():
            xb_copy().start()

        @pl.when(s0 == 4)
        def _():
            xb_copy().wait()


    def step(s, order, o_scr, o_in=None):
        static = isinstance(s, int)
        slot = s & (NS - 1)
        qs = s & (NQ - 1)
        o_in = o_scr if o_in is None else o_in

        def qk(b):
            rows = pl.ds(b * SQ, SQ)
            qb = jnp.concatenate([q_buf[qs, rows, 0:DH], q_buf[qs, rows, DH:2 * DH]], axis=0)
            return lax.dot_general(qb, k_buf[slot, b], NT, preferred_element_type=jnp.float32)

        def pv(b, sc):
            rows = pl.ds(b * SQ, SQ)
            m = jnp.max(sc, axis=1, keepdims=True)
            p = jnp.exp2(sc - m)
            l = jnp.sum(p, axis=1, keepdims=True)
            rl = pl.reciprocal(l, approx=True)
            rl = rl * (2.0 - l * rl)
            o = jnp.dot(p.astype(jnp.bfloat16), v_buf[slot, b], preferred_element_type=jnp.float32)
            o = (o * rl).astype(jnp.bfloat16)
            o_scr[rows, 0:DH] = o[0:SQ]
            o_scr[rows, DH:2 * DH] = o[SQ:2 * SQ]

        def outproj(c0, n):
            if static:
                arow = pl.ds(((s - OD) >> 4) * D, D)
            else:
                arow = pl.ds(pl.multiple_of(lax.shift_right_logical(s - OD, 4) * D, 64), D)
            part = lax.dot_general(wo_buf[(s - OD) & (NS - 1)], o_in[pl.ds(c0, n), :], NT,
                                   preferred_element_type=jnp.float32)
            acc[arow, pl.ds(c0, n)] += part

        def fin_hi(b):
            ob_hi[pl.ds(b * SQ, SQ), :] = acc[LO:2 * D, pl.ds(b * SQ, SQ)].astype(jnp.bfloat16).T
            if (b + 1) % HCH == 0:
                hi_copy(b // HCH).start()

        def qhalf(h):
            t = s + AHEAD
            tr = t >> 4 if static else lax.shift_right_logical(t, 4)
            qproj(tr, t & (NW - 1), t & (NQ - 1), h * (M // 2), M // 2)

        def background(n):
            for j in range(n):
                bb = (s + j + 4) & 7
                xpose(jnp.where(s >= 4, 1, 0), jnp.where((s >= 4) & (s < 12), 1, 2), bb)

        def fin_lo():
            h = s - (NSTEP - AHEAD)
            nb = B // AHEAD
            for j in range(nb):
                if static:
                    rows = pl.ds((nb * h + j) * SQ, SQ)
                else:
                    rows = pl.ds(pl.multiple_of((nb * h + j) * SQ, SQ), SQ)
                ob_lo[rows, :] = acc[0:LO, rows].astype(jnp.bfloat16).T

        scs = {}
        for tok in order.split():
            k, i = tok[0], int(tok[1:]) if len(tok) > 1 else None
            if k == "Q":
                scs[i] = qk(i)
            elif k == "P":
                pv(i, scs.pop(i))
            elif k == "O":
                outproj(i * 256, 256)
            elif k == "F":
                fin_hi(2 * i)
                fin_hi(2 * i + 1)
            elif k == "X":
                qhalf(i)
            elif k == "D":
                prefetch(s)
            elif k == "B":
                background(i or 1)
            elif k == "A":
                fin_lo()
            elif k == "W" and i is not None:
                kv0_copy(0, i).wait()
                kv0_copy(1, i).wait()

    def first_copies():
        xa_copy(0).start()
        wq_copy(0, 0, 0).start()
        xa_copy(1).start()
        for t in range(1, AHEAD):
            wq_copy(0, t, t).start()
        kv0_copy(0, 0).start()
        kv0_copy(1, 0).start()
        kv0_copy(0, 1).start()
        kv0_copy(1, 1).start()
        wq_copy(0, AHEAD, AHEAD).start()
        for t in range(1, U):
            k_copy(0, t, t).start()
            v_copy(0, t, t).start()
            wq_copy(0, t + AHEAD, t + AHEAD).start()
        for t in range(0, U - OD):
            wo_copy(0, t, t).start()

    with scope("p0"):
        first_copies()
    with scope("p1"):
        xa_copy(0).wait()
        for b in range(4):
            xpose(0, 0, b)
    with scope("p2"):
        wq_copy(0, 0, 0).wait()
        qproj(0, 0, 0, 0, M // 2)
    with scope("p3"):
        xa_copy(1).wait()
        for t in range(1, AHEAD):
            wq_copy(0, 0, t).wait()
        for b in range(4, 8):
            xpose(0, 0, b)
        qproj(0, 1, 1, 0, M // 2)
        qproj(0, 0, 0, M // 2, M // 2)
        qproj(0, 1, 1, M // 2, M // 2)
        acc[...] = jnp.zeros(acc.shape, jnp.float32)
        for t in range(2, AHEAD):
            qproj(0, t, t, 0, M // 2)
            qproj(0, t, t, M // 2, M // 2)
    for s in range(NP):
        o = ORDER_0 if s == 0 else (ORDER_P if s < OD else ORDER.replace("B2", "").replace("B", ""))
        with scope("wait"):
            waits(s, o)
        with scope("body%d" % s):
            step(s, o, o_bufs[s % U])

    with scope("loop"):
        def main_body(i, c):
            s0 = NP + i * U
            with scope("wait"):
                for u in range(U):
                    waits(s0 + u, ORDER)
                events(s0)
            for u in range(U):
                step(s0 + u, (ORDER, ORDER1)[u], o_bufs[u], o_bufs[(u - OD) % U])
            return c
        lax.fori_loop(0, (NSTEP - AHEAD - NP) // U, main_body, 0)

    with scope("tail"):
        if U == 1:
            def tail_body(s, c):
                with scope("wait"):
                    waits(s, ORDER_T)
                step(s, ORDER_T, o_a)
                return c
            lax.fori_loop(NSTEP - AHEAD, NSTEP, tail_body, 0)
        else:
            def tail_body(i, c):
                s0 = NSTEP - AHEAD + i * U
                with scope("wait"):
                    for u in range(U):
                        waits(s0 + u, ORDER_T)
                for u in range(U):
                    step(s0 + u, ORDER_T, o_bufs[u], o_bufs[(u - OD) % U])
                return c
            if AHEAD == U:
                tail_body(0, 0)
            else:
                lax.fori_loop(0, AHEAD // U, tail_body, 0)

    with scope("wait"):
        lo_copy().start()
        for s in range(NSTEP, NSTEP + OD):
            waits(s, "O")
    with scope("last"):
        for c in range(4):
            for s in range(NSTEP, NSTEP + OD):
                step(s, "O%d" % c, o_bufs[(s - OD) % U])
            step(NSTEP, "F%d" % c, o_a)
    with scope("fin"):
        lo_copy().wait()
        for b in range(B // HCH):
            hi_copy(b).wait()


@jax.jit
def pallas_concat_heads__gqa_block_cached__gqa_block_cached__near_ridge_kernel(
        A_x, A_k_cache, A_v_cache, A_wq, A_wo, B_x, B_k_cache, B_v_cache, B_wq, B_wo):
    hbm = pl.BlockSpec(memory_space=pltpu.HBM)
    flags = {k: True for k in FLAGS.split(",") if k} or None
    out = pl.pallas_call(
        _kernel,
        out_shape=jax.ShapeDtypeStruct((M, 2 * D), jnp.bfloat16),
        in_specs=[hbm] * 10,
        out_specs=hbm,
        scratch_shapes=[
            pltpu.VMEM((2, B, D, SQ), jnp.bfloat16),
            pltpu.VMEM((3, M, D), jnp.bfloat16),
            pltpu.VMEM((NW, D, GW), jnp.bfloat16),
            pltpu.VMEM((NS, B, SK, DH), jnp.bfloat16),
            pltpu.VMEM((NS, B, SK, DH), jnp.bfloat16),
            pltpu.VMEM((NS, D, GW), jnp.bfloat16),
            pltpu.VMEM((NQ, M, GW), jnp.bfloat16),
            pltpu.VMEM((M, GW), jnp.bfloat16),
            pltpu.VMEM((M, GW), jnp.bfloat16),
            pltpu.VMEM((2 * D, M), jnp.float32),
            pltpu.VMEM((M, LO), jnp.bfloat16),
            pltpu.VMEM((M, HI), jnp.bfloat16),
            pltpu.SemaphoreType.DMA((16 + NW + 3 * NS,)),
        ],
        compiler_params=pltpu.CompilerParams(vmem_limit_bytes=100 * 1024 * 1024, flags=flags,
                                             disable_bounds_checks=True),
        name="gqa2",
    )(A_x.transpose(0, 2, 1), A_k_cache, A_v_cache, A_wq, A_wo.T,
      B_x.transpose(0, 2, 1), B_k_cache, B_v_cache, B_wq, B_wo.T)
    return out.reshape(B, SQ, 2 * D)
```

```python
import jax
import jax.numpy as jnp
from jax import lax
import jax.experimental.pallas as pl
import jax.experimental.pallas.tpu as pltpu

B, SQ, D = 8, 128, 576
HKV, SK, DH = 16, 512, 128
M = B * SQ
GW = 2 * DH
NSTEP = 2 * HKV
U = 2
NS = 2 * U
LO = 512
HI = 2 * D - LO
QSCALE = (DH ** -0.5) * 1.4426950408889634
NT = (((1,), (1,)), ((), ()))

ATT = "Q0 Q1 P0 Q2 P1 Q3 P2 Q4 P3 Q5 P4 Q6 P5 Q7 P6 P7"
ORDER_0 = "D W0 Q0 Q1 P0 Q2 P1 Q3 P2 W1 Q4 P3 Q5 P4 Q6 P5 Q7 P6 P7 X0 X1"
ORDER_1 = "D " + ATT + " X0 X1"
ORDER = "O0 D B O1 O2 O3 " + ATT + " X0 X1"
ORDER_T = "O0 D O1 A O2 O3 " + ATT


def _kernel(xa, ka, va, wqa, woa, xb, kb, vb, wqb, wob, out,
            xt_buf, x_buf, w_buf, kv_buf, q_buf, o_a, o_b, acc, ob_lo, ob_hi, sems):
    srcs = ((xa, ka, va, wqa, woa), (xb, kb, vb, wqb, wob))
    o_bufs = (o_a, o_b)
    S_X, S_LO, S_H, S_W, S_P, S_G, S_HI = 0, 3, 4, 8, 11, 13, 17

    def cols(g):
        return pl.ds(g * GW, GW) if isinstance(g, int) else pl.ds(pl.multiple_of(g * GW, GW), GW)

    def xa_copy(h):
        return pltpu.make_async_copy(xa.at[pl.ds(4 * h, 4)], xt_buf.at[0, pl.ds(4 * h, 4)], sems.at[S_X + h])

    def xb_copy():
        return pltpu.make_async_copy(xb, xt_buf.at[1], sems.at[S_X + 2])

    def kv0_copy(which, h):
        src = (ka, va)[which]
        return pltpu.make_async_copy(src.at[pl.ds(4 * h, 4), 0], kv_buf.at[0, which, pl.ds(4 * h, 4)],
                                     sems.at[S_H + 2 * h + which])

    def packet_copy(which, r, g, slot, sem):
        if which < 2:
            return pltpu.make_async_copy(srcs[r][1 + which].at[:, g], kv_buf.at[slot, which], sem)
        return pltpu.make_async_copy(srcs[r][1 + which].at[:, cols(g)], w_buf.at[slot, which - 2], sem)

    def packet_start(s, base):
        for which in range(4):
            t = s + (0, 0, 2, -2)[which]
            sem = sems.at[base + which // 2]
            if isinstance(s, int):
                if 0 <= t < NSTEP:
                    packet_copy(which, t >> 4, t & (HKV - 1), s & (NS - 1), sem).start()
                continue
            for rr in range(2):
                @pl.when(lax.shift_right_logical(t, 4) == rr)
                def _():
                    packet_copy(which, rr, t & (HKV - 1), s & (NS - 1), sem).start()

    def group_base(s):
        return S_G + (s & 2)

    def wait_region(ref, i):
        pltpu.make_async_copy(ref, ref, sems.at[i]).wait()

    def lo_copy():
        return pltpu.make_async_copy(ob_lo, out.at[:, pl.ds(0, LO)], sems.at[S_LO])

    def hi_copy(b):
        rows = pl.ds(b * SQ, SQ)
        return pltpu.make_async_copy(ob_hi.at[rows], out.at[rows, pl.ds(LO, HI)], sems.at[S_HI + b])

    def xpose(src_r, dst_r, b):
        rows = pl.ds(b * SQ, SQ) if isinstance(b, int) else pl.ds(pl.multiple_of(b * SQ, SQ), SQ)
        x_buf[dst_r, rows, :] = xt_buf[src_r, b].T

    def qproj(t, h):
        r = t >> 4 if isinstance(t, int) else lax.shift_right_logical(t, 4)
        rows = pl.ds(h * (M // 2), M // 2)
        q = jnp.dot(x_buf[r, rows, :], w_buf[(t - 2) & (NS - 1), 0], preferred_element_type=jnp.float32)
        q_buf[t & (NS - 1), rows, :] = (q * QSCALE).astype(jnp.bfloat16)

    def step(s, order, o_scr):
        static = isinstance(s, int)
        slot = s & (NS - 1)

        def qk(b):
            rows = pl.ds(b * SQ, SQ)
            qb = jnp.concatenate([q_buf[slot, rows, 0:DH], q_buf[slot, rows, DH:2 * DH]], axis=0)
            return lax.dot_general(qb, kv_buf[slot, 0, b], NT, preferred_element_type=jnp.float32)

        def pv(b, sc):
            rows = pl.ds(b * SQ, SQ)
            m = jnp.max(sc, axis=1, keepdims=True)
            p = jnp.exp2(sc - m)
            l = jnp.sum(p, axis=1, keepdims=True)
            rl = pl.reciprocal(l, approx=True)
            rl = rl * (2.0 - l * rl)
            o = jnp.dot(p.astype(jnp.bfloat16), kv_buf[slot, 1, b], preferred_element_type=jnp.float32)
            o = (o * rl).astype(jnp.bfloat16)
            o_scr[rows, 0:DH] = o[0:SQ]
            o_scr[rows, DH:2 * DH] = o[SQ:2 * SQ]

        def outproj(c):
            if static:
                arow = pl.ds(((s - 2) >> 4) * D, D)
            else:
                arow = pl.ds(pl.multiple_of(lax.shift_right_logical(s - 2, 4) * D, 64), D)
            tok = pl.ds(c * 2 * SQ, 2 * SQ)
            acc[arow, tok] += lax.dot_general(w_buf[slot, 1], o_scr[tok, :], NT,
                                              preferred_element_type=jnp.float32)

        scs = {}
        for tok in order.split():
            k, i = tok[0], int(tok[1:]) if len(tok) > 1 else None
            if k == "Q":
                scs[i] = qk(i)
            elif k == "P":
                pv(i, scs.pop(i))
            elif k == "O":
                outproj(i)
            elif k == "X":
                qproj(s + 2, i)
            elif k == "D":
                packet_start(s + U, group_base(s + U))
            elif k == "B":
                xpose(jnp.where(s >= 4, 1, 0), jnp.where((s >= 4) & (s < 12), 1, 2), (s + 4) & 7)
            elif k == "A":
                for b in range(4 * (s - (NSTEP - 2)), 4 * (s - (NSTEP - 2)) + 4):
                    rows = pl.ds(b * SQ, SQ)
                    ob_lo[rows, :] = acc[0:LO, rows].astype(jnp.bfloat16).T
            elif k == "F":
                for b in (2 * i, 2 * i + 1):
                    rows = pl.ds(b * SQ, SQ)
                    ob_hi[rows, :] = acc[LO:2 * D, rows].astype(jnp.bfloat16).T
                    hi_copy(b).start()
            elif k == "W":
                kv0_copy(0, i).wait()
                kv0_copy(1, i).wait()
                if i == 1:
                    wait_region(w_buf.at[0, 0], S_W + 2)

    xa_copy(0).start()
    packet_copy(2, 0, 0, 2, sems.at[S_W]).start()
    xa_copy(1).start()
    packet_copy(2, 0, 1, 3, sems.at[S_W + 1]).start()
    for h in range(2):
        kv0_copy(0, h).start()
        kv0_copy(1, h).start()
    packet_copy(2, 0, 2, 0, sems.at[S_W + 2]).start()
    packet_start(1, S_P)

    xa_copy(0).wait()
    for b in range(4):
        xpose(0, 0, b)
    wait_region(w_buf.at[2, 0], S_W)
    qproj(0, 0)
    xa_copy(1).wait()
    wait_region(w_buf.at[3, 0], S_W + 1)
    for b in range(4, 8):
        xpose(0, 0, b)
    qproj(1, 0)
    qproj(0, 1)
    qproj(1, 1)
    acc[...] = jnp.zeros(acc.shape, jnp.float32)
    step(0, ORDER_0, o_a)
    wait_region(kv_buf.at[1], S_P)
    wait_region(w_buf.at[1, 0], S_P + 1)
    step(1, ORDER_1, o_b)

    def main_body(i, c):
        s0 = U + i * U
        pair = pl.ds(pl.multiple_of(s0 & (NS - 1), U), U)
        wait_region(kv_buf.at[pair], group_base(s0))
        wait_region(w_buf.at[pair], group_base(s0) + 1)

        @pl.when(s0 == 2)
        def _():
            xb_copy().start()

        @pl.when(s0 == 4)
        def _():
            xb_copy().wait()

        for u in range(U):
            step(s0 + u, ORDER, o_bufs[u])
        return c

    lax.fori_loop(0, (NSTEP - 2 - U) // U, main_body, 0)

    s0 = NSTEP - 2
    pair = pl.ds(s0 & (NS - 1), U)
    wait_region(kv_buf.at[pair], group_base(s0))
    wait_region(w_buf.at[pair, 1], group_base(s0) + 1)
    for u in range(U):
        step(s0 + u, ORDER_T, o_bufs[u])

    lo_copy().start()
    wait_region(w_buf.at[pl.ds(NSTEP & (NS - 1), U), 1], group_base(NSTEP) + 1)
    for c in range(4):
        for u in range(U):
            step(NSTEP + u, "O%d" % c, o_bufs[u])
        step(NSTEP, "F%d" % c, o_a)
        if c == 2:
            lo_copy().wait()
    for b in range(B):
        hi_copy(b).wait()


@jax.jit
def pallas_concat_heads__gqa_block_cached__gqa_block_cached__near_ridge_kernel(
    A_x: jax.Array,
    A_k_cache: jax.Array,
    A_v_cache: jax.Array,
    A_wq: jax.Array,
    A_wo: jax.Array,
    B_x: jax.Array,
    B_k_cache: jax.Array,
    B_v_cache: jax.Array,
    B_wq: jax.Array,
    B_wo: jax.Array,
):
    hbm = pl.BlockSpec(memory_space=pltpu.HBM)
    out = pl.pallas_call(
        _kernel,
        out_shape=jax.ShapeDtypeStruct((M, 2 * D), jnp.bfloat16),
        in_specs=[hbm] * 10,
        out_specs=hbm,
        scratch_shapes=[
            pltpu.VMEM((2, B, D, SQ), jnp.bfloat16),
            pltpu.VMEM((3, M, D), jnp.bfloat16),
            pltpu.VMEM((NS, 2, D, GW), jnp.bfloat16),
            pltpu.VMEM((NS, 2, B, SK, DH), jnp.bfloat16),
            pltpu.VMEM((NS, M, GW), jnp.bfloat16),
            pltpu.VMEM((M, GW), jnp.bfloat16),
            pltpu.VMEM((M, GW), jnp.bfloat16),
            pltpu.VMEM((2 * D, M), jnp.float32),
            pltpu.VMEM((M, LO), jnp.bfloat16),
            pltpu.VMEM((M, HI), jnp.bfloat16),
            pltpu.SemaphoreType.DMA((17 + B,)),
        ],
        compiler_params=pltpu.CompilerParams(vmem_limit_bytes=100 * 1024 * 1024,
                                             disable_bounds_checks=True),
    )(A_x.transpose(0, 2, 1), A_k_cache, A_v_cache, A_wq, A_wo.T,
      B_x.transpose(0, 2, 1), B_k_cache, B_v_cache, B_wq, B_wo.T)
    return out.reshape(B, SQ, 2 * D)
```
